```python
import jax
import jax.numpy as jnp

def _softmax(x, axis=-1):
    return jax.nn.softmax(x, axis=axis)

def _gelu(x):
    return jax.nn.gelu(x, approximate=True)

def _silu(x):
    return jax.nn.silu(x)

def _sigmoid(x):
    return jax.nn.sigmoid(x)

def _layernorm(x, axis=-1, eps=1e-05):
    m = jnp.mean(x, axis=axis, keepdims=True)
    v = jnp.var(x, axis=axis, keepdims=True)
    return (x - m) / jnp.sqrt(v + eps)

def _scatter_add(tgt, idx, src, axis=0):
    return tgt.at[idx].add(src)

def _segment_sum(src, seg, n):
    return jax.ops.segment_sum(src, seg, n)

class _Rng:

    def __init__(self, key):
        self._k = key

    def _next(self):
        self._k, sub = jax.random.split(self._k)
        return sub

    def normal(self, shape):
        return jax.random.normal(self._next(), shape, dtype=jnp.bfloat16)

    def randint(self, lo, hi, shape):
        return jax.random.randint(self._next(), shape, lo, hi, dtype=jnp.int32)

    def uniform(self, shape, lo=0.0, hi=1.0):
        return jax.random.uniform(self._next(), shape, jnp.bfloat16, lo, hi)

    def permutation(self, n):
        return jax.random.permutation(self._next(), n)
kernel_name = 'adaLN_cond__mha_block_cached__moe_arch_mod__prompt'

def setup_inputs():
    _rng = _Rng(jax.random.key(int.from_bytes(__import__("os").urandom(4), "little")))
    _w = lambda a: (lambda t: t.astype(jnp.bfloat16) if jnp.issubdtype(t.dtype, jnp.floating) else t)(jnp.asarray(a))

    def _A_setup():
        B, Sq, D = (1, 2048, 1024)
        H, Sk, Dh = (32, 2048, 128)
        return {'x': _w((lambda *s: _rng.normal(s) * 0.05)(B, Sq, D)), 'k_cache': _w((lambda *s: _rng.normal(s) * 0.05)(B, H, Sk, Dh)), 'v_cache': _w((lambda *s: _rng.normal(s) * 0.05)(B, H, Sk, Dh)), 'wq': _w((lambda *s: _rng.normal(s) * 0.05)(D, H * Dh) * D ** (-0.5)), 'wo': _w((lambda *s: _rng.normal(s) * 0.05)(H * Dh, D) * (H * Dh) ** (-0.5))}
    _A_in = _A_setup()

    def _B_setup():
        B, S, D, F, C = (1, 2048, 1024, 3584, 2)
        return {'x': _w((lambda *s: _rng.normal(s) * 0.05)(B, S, D)), 'w_r': _w((lambda *s: _rng.normal(s) * 0.05)(D)), 'w_gate': _w((lambda *s: _rng.normal(s) * 0.05)(D, F)), 'w_up': _w((lambda *s: _rng.normal(s) * 0.05)(D, F)), 'w_down': _w((lambda *s: _rng.normal(s) * 0.05)(F, D))}
    _B_in = _B_setup()
    return {'A_x': _A_in['x'], 'A_k_cache': _A_in['k_cache'], 'A_v_cache': _A_in['v_cache'], 'A_wq': _A_in['wq'], 'A_wo': _A_in['wo'], 'B_x': _B_in['x'], 'B_w_r': _B_in['w_r'], 'B_w_gate': _B_in['w_gate'], 'B_w_up': _B_in['w_up'], 'B_w_down': _B_in['w_down'], 'c': _w((lambda *s: _rng.normal(s) * 0.05)(1, 1024)), 'w_mod': _w((lambda *s: _rng.normal(s) * 0.05)(1024, 6 * 1024) * 1024 ** (-0.5))}

def reference(A_x, A_k_cache, A_v_cache, A_wq, A_wo, B_x, B_w_r, B_w_gate, B_w_up, B_w_down, c, w_mod):

    def _A_ref(x, k_cache, v_cache, wq, wo):
        B, Sq, D = x.shape
        H, Dh = (32, 128)
        q = (lambda x, *d: x.transpose(*d))((x @ wq).reshape(B, Sq, H, Dh), 0, 2, 1, 3)
        scores = jnp.einsum('bhqd,bhkd->bhqk', q, k_cache) * Dh ** (-0.5)
        p = _softmax(scores, axis=-1)
        o = jnp.einsum('bhqk,bhkd->bhqd', p, v_cache)
        return (lambda x, *d: x.transpose(*d))(o, 0, 2, 1, 3).reshape(B, Sq, H * Dh) @ wo

    def _B_ref(x, w_r, w_gate, w_up, w_down):
        B, S, D = x.shape
        C = 2
        r = x @ w_r
        idx = jnp.argsort(-r, axis=-1)[:, :C]
        idx_e = jnp.repeat(idx.reshape(B, C, 1), D, axis=2)
        x_sel = jnp.take_along_axis(x, idx_e, axis=1)
        g = _silu(x_sel @ w_gate)
        u = x_sel @ w_up
        y = g * u @ w_down
        r_sel = _sigmoid(jnp.take_along_axis(r, idx, axis=1))
        y = y * r_sel.reshape(B, C, 1)
        b_off = (jnp.arange(B) * S).reshape(B, 1)
        flat_idx = (idx + b_off).reshape(B * C)
        zero = (x * 0.0).reshape(B * S, D)
        upd = _scatter_add(zero, flat_idx, y.reshape(B * C, D), axis=0)
        return x + upd.reshape(B, S, D)
    x = A_x
    mod = (_silu(c) @ w_mod).reshape(c.shape[0], 6, 1, -1)
    sa, ca, ga, sb, cb, gb = (mod[:, 0].copy(), mod[:, 1].copy(), mod[:, 2].copy(), mod[:, 3].copy(), mod[:, 4].copy(), mod[:, 5].copy())
    h = _layernorm(x, axis=-1) * (1 + ca) + sa
    x = x + ga * _A_ref(h, A_k_cache, A_v_cache, A_wq, A_wo)
    h = _layernorm(x, axis=-1) * (1 + cb) + sb
    x = x + gb * _B_ref(h, B_w_r, B_w_gate, B_w_up, B_w_down)
    return x
```

```python
import functools
import math

import jax
import jax.numpy as jnp
from jax import lax
import jax.experimental.pallas as pl
import jax.experimental.pallas.tpu as pltpu

S = 2048
D = 1024
H = 32
DH = 128
F = 3584
EPS = 1e-5
QSCALE = (DH ** -0.5) * math.log2(math.e)

BQ = 256
RB = 256
XCH = 4
NEG = -3.0e38

BF = jnp.bfloat16
F32 = jnp.float32
NT = (((1,), (1,)), ((), ()))


def _ln(x):
    m = jnp.mean(x, axis=-1, keepdims=True)
    d = x - m
    v = jnp.mean(d * d, axis=-1, keepdims=True)
    return d * lax.rsqrt(v + EPS)


def _kernel(x_hbm, k_hbm, v_hbm, wq_hbm, wo_hbm, wr_hbm, wg_hbm, wu_hbm, wd_hbm,
            c_hbm, wm_hbm, out_hbm,
            x_buf, h_buf, wq_buf, k_buf, v_buf, q_buf, o_buf, wo_buf, wg_buf,
            wu_buf, wd_buf, wm_buf, x1_buf, r_buf, mod_buf, c_buf, wr_buf,
            fix_buf, sem_misc, sem_x, sem_wm, sem_kv, sem_wq, sem_bg, sem_out,
            sem_fix):
    def cp_c():
        return pltpu.make_async_copy(c_hbm, c_buf, sem_misc.at[0])

    def cp_wr():
        return pltpu.make_async_copy(wr_hbm, wr_buf, sem_misc.at[1])

    def cp_wm(j):
        cols = pl.ds(j * 512, 512)
        return pltpu.make_async_copy(wm_hbm.at[:, cols], wm_buf.at[:, cols], sem_wm.at[j])

    XR = S // XCH

    def cp_x(j):
        rows = pl.ds(j * XR, XR)
        return pltpu.make_async_copy(x_hbm.at[rows, :], x_buf.at[rows, :], sem_x.at[j])

    def cp_k(h, slot):
        return pltpu.make_async_copy(k_hbm.at[h], k_buf.at[slot], sem_kv.at[0, slot])

    def cp_v(h, slot):
        return pltpu.make_async_copy(v_hbm.at[h], v_buf.at[slot], sem_kv.at[1, slot])

    def cp_wq(h, slot):
        cols = pl.ds(pl.multiple_of(h * DH, DH), DH)
        return pltpu.make_async_copy(wq_hbm.at[:, cols], wq_buf.at[slot], sem_wq.at[slot])

    def bg_copies(h):
        r128 = pl.ds(pl.multiple_of(h * 128, 128), 128)
        r32 = pl.ds(pl.multiple_of(h * 32, 32), 32)
        r112 = pl.ds(pl.multiple_of(h * 112, 16), 112)
        cols = pl.ds(2048, 4096)
        return [
            pltpu.make_async_copy(wo_hbm.at[r128, :], wo_buf.at[r128, :], sem_bg.at[0]),
            pltpu.make_async_copy(wm_hbm.at[r32, cols], wm_buf.at[r32, cols], sem_bg.at[1]),
            pltpu.make_async_copy(wg_hbm.at[r32, :], wg_buf.at[r32, :], sem_bg.at[2]),
            pltpu.make_async_copy(wu_hbm.at[r32, :], wu_buf.at[r32, :], sem_bg.at[3]),
            pltpu.make_async_copy(wd_hbm.at[r112, :], wd_buf.at[r112, :], sem_bg.at[4]),
        ]

    def bg_wait_all():
        cols = pl.ds(2048, 4096)
        pltpu.make_async_copy(wo_hbm, wo_buf, sem_bg.at[0]).wait()
        pltpu.make_async_copy(wm_hbm.at[:, cols], wm_buf.at[:, cols], sem_bg.at[1]).wait()
        pltpu.make_async_copy(wg_hbm, wg_buf, sem_bg.at[2]).wait()
        pltpu.make_async_copy(wu_hbm, wu_buf, sem_bg.at[3]).wait()
        pltpu.make_async_copy(wd_hbm, wd_buf, sem_bg.at[4]).wait()

    cp_c().start()
    for j in range(4):
        cp_wm(j).start()
    cp_wq(0, 0).start()
    for j in range(XCH):
        cp_x(j).start()
    cp_k(0, 0).start()
    cp_v(0, 0).start()
    cp_wq(1, 1).start()
    cp_wr().start()

    cp_c().wait()
    cf = c_buf[...].astype(F32)
    sc = (cf * jax.nn.sigmoid(cf)).astype(BF)
    sc16 = jnp.broadcast_to(sc, (16, D))
    for j in range(4):
        cp_wm(j).wait()
        mj = jnp.dot(sc16, wm_buf[:, j * 512:(j + 1) * 512], preferred_element_type=F32)
        mod_buf[:, j * 512:(j + 1) * 512] = mj[0:8, :]

    cp_wq(0, 0).wait()
    for j in range(XCH):
        cp_x(j).wait()
        for t in range(XR // RB):
            rows = pl.ds(j * XR + t * RB, RB)
            n = _ln(x_buf[rows, :].astype(F32))
            h = n * (1.0 + mod_buf[0:1, D:2 * D]) + mod_buf[0:1, 0:D]
            hb = h.astype(BF)
            h_buf[rows, :] = hb
            q = jnp.dot(hb, wq_buf[0], preferred_element_type=F32)
            q_buf[0, rows, :] = (q * QSCALE).astype(BF)

    def qproj(slot):
        q = jnp.dot(h_buf[...], wq_buf[slot], preferred_element_type=F32)
        q_buf[slot, :, :] = (q * QSCALE).astype(BF)

    def attention(h, slot):
        for i in range(S // BQ):
            rows = pl.ds(i * BQ, BQ)
            q = q_buf[slot, rows, :]
            s = lax.dot_general(q, k_buf[slot], NT, preferred_element_type=F32)
            m = jnp.max(s, axis=1, keepdims=True)
            p = jnp.exp2(s - m)
            l = jnp.sum(p, axis=1, keepdims=True)
            o = jnp.dot(p.astype(BF), v_buf[slot], preferred_element_type=F32)
            o_buf[h, rows, :] = (o * (1.0 / l)).astype(BF)

    def head_body(h, carry):
        slot = lax.rem(h, 2)
        nslot = 1 - slot
        cp_k(h, slot).wait()
        cp_v(h, slot).wait()
        cp_wq(h + 1, nslot).wait()
        cp_k(h + 1, nslot).start()
        cp_v(h + 1, nslot).start()
        cp_wq(jnp.minimum(h + 2, H - 1), slot).start()
        for cpy in bg_copies(h):
            cpy.start()
        attention(h, slot)
        qproj(nslot)
        return carry

    lax.fori_loop(0, H - 1, head_body, 0)

    cp_wq(H - 1, (H - 2) % 2).wait()
    cp_k(H - 1, (H - 1) % 2).wait()
    cp_v(H - 1, (H - 1) % 2).wait()
    for cpy in bg_copies(H - 1):
        cpy.start()
    attention(H - 1, (H - 1) % 2)

    bg_wait_all()
    cp_wr().wait()
    for j in range(4, 12):
        mj = jnp.dot(sc16, wm_buf[:, j * 512:(j + 1) * 512], preferred_element_type=F32)
        mod_buf[:, j * 512:(j + 1) * 512] = mj[0:8, :]

    def mod(i):
        return mod_buf[0:1, i * D:(i + 1) * D]

    def cp_out(i):
        rows = pl.ds(i * RB, RB)
        return pltpu.make_async_copy(h_buf.at[rows, :], out_hbm.at[rows, :], sem_out.at[i])

    def h2_of(x1):
        return (_ln(x1) * (1.0 + mod(4)) + mod(3)).astype(BF).astype(F32)

    wr = wr_buf[...].astype(F32)
    for i in range(S // RB):
        rows = pl.ds(i * RB, RB)
        oc = jnp.concatenate([o_buf[hh, rows, :] for hh in range(H)], axis=1)
        y = jnp.dot(oc, wo_buf[...], preferred_element_type=F32)
        x1 = x_buf[rows, :].astype(F32) + mod(2) * y
        x1_buf[rows, :] = x1
        h2 = h2_of(x1)
        acc = h2[:, 0:128] * wr[0:1, :]
        for j in range(1, 8):
            acc = acc + h2[:, j * 128:(j + 1) * 128] * wr[j:j + 1, :]
        r = jnp.sum(acc, axis=1, keepdims=True).astype(BF).astype(F32)
        r_buf[rows, :] = jnp.broadcast_to(r, (RB, 128))
        h_buf[rows, :] = (x1 + mod(5) * h2).astype(BF)
        cp_out(i).start()

    r_all = r_buf[...]
    ridx = lax.broadcasted_iota(jnp.int32, (S, 128), 0)
    m1 = jnp.max(r_all, axis=0, keepdims=True)
    i1 = jnp.min(jnp.where(r_all == m1, ridx, S), axis=0, keepdims=True)
    r_m = jnp.where(ridx == i1, NEG, r_all)
    m2 = jnp.max(r_m, axis=0, keepdims=True)
    i2 = jnp.min(jnp.where(jnp.logical_and(r_m == m2, ridx != i1), ridx, S), axis=0, keepdims=True)
    idx1 = jnp.clip(jnp.max(i1), 0, S - 1)
    idx2 = jnp.clip(jnp.max(i2), 0, S - 1)

    g1 = pl.multiple_of((idx1 // 16) * 16, 16)
    g2 = pl.multiple_of((idx2 // 16) * 16, 16)
    x1_g1 = x1_buf[pl.ds(g1, 16), :]
    x1_g2 = x1_buf[pl.ds(g2, 16), :]
    h2_g1 = h2_of(x1_g1)
    h2_g2 = h2_of(x1_g2)
    ri = lax.broadcasted_iota(jnp.int32, (16, D), 0)
    sel11 = ri == (idx1 - g1)
    sel22 = ri == (idx2 - g2)
    xs1 = jnp.sum(jnp.where(sel11, h2_g1, 0.0), axis=0, keepdims=True)
    xs2 = jnp.sum(jnp.where(sel22, h2_g2, 0.0), axis=0, keepdims=True)
    xsel = jnp.where(ri == 0, xs1, jnp.where(ri == 1, xs2, 0.0)).astype(BF)

    g = jnp.dot(xsel, wg_buf[...], preferred_element_type=F32)
    u = jnp.dot(xsel, wu_buf[...], preferred_element_type=F32)
    a = (g * jax.nn.sigmoid(g) * u).astype(BF)
    y = jnp.dot(a, wd_buf[...], preferred_element_type=F32)
    w1 = jax.nn.sigmoid(m1[:, 0:1])
    w2 = jax.nn.sigmoid(m2[:, 0:1])
    y1 = y[0:1, :] * w1
    y2 = y[1:2, :] * w2

    def fixed(gbase, x1_g, h2_g):
        upd = jnp.where(ri == (idx1 - gbase), y1, 0.0) + jnp.where(ri == (idx2 - gbase), y2, 0.0)
        return (x1_g + mod(5) * (h2_g + upd)).astype(BF)

    fix_buf[0] = fixed(g1, x1_g1, h2_g1)
    fix_buf[1] = fixed(g2, x1_g2, h2_g2)

    for i in range(S // RB):
        cp_out(i).wait()

    cp1 = pltpu.make_async_copy(fix_buf.at[0], out_hbm.at[pl.ds(g1, 16), :], sem_fix.at[0])
    cp1.start()

    @pl.when(g1 != g2)
    def _():
        cp2 = pltpu.make_async_copy(fix_buf.at[1], out_hbm.at[pl.ds(g2, 16), :], sem_fix.at[1])
        cp2.start()
        cp2.wait()

    cp1.wait()


@jax.jit
def pallas_adaLN_cond__mha_block_cached__moe_arch_mod__prompt_kernel(
    A_x, A_k_cache, A_v_cache, A_wq, A_wo, B_x, B_w_r, B_w_gate, B_w_up, B_w_down, c, w_mod,
):
    del B_x
    x = A_x.reshape(S, D)
    k = A_k_cache.reshape(H, S, DH)
    v = A_v_cache.reshape(H, S, DH)
    wr = B_w_r.reshape(8, 128)
    any_spec = pl.BlockSpec(memory_space=pl.ANY)
    scratch = [
        pltpu.VMEM((S, D), BF),
        pltpu.VMEM((S, D), BF),
        pltpu.VMEM((2, D, DH), BF),
        pltpu.VMEM((2, S, DH), BF),
        pltpu.VMEM((2, S, DH), BF),
        pltpu.VMEM((2, S, DH), BF),
        pltpu.VMEM((H, S, DH), BF),
        pltpu.VMEM((H * DH, D), BF),
        pltpu.VMEM((D, F), BF),
        pltpu.VMEM((D, F), BF),
        pltpu.VMEM((F, D), BF),
        pltpu.VMEM((D, 6 * D), BF),
        pltpu.VMEM((S, D), F32),
        pltpu.VMEM((S, 128), F32),
        pltpu.VMEM((8, 6 * D), F32),
        pltpu.VMEM((1, D), BF),
        pltpu.VMEM((8, 128), BF),
        pltpu.VMEM((2, 16, D), BF),
        pltpu.SemaphoreType.DMA((2,)),
        pltpu.SemaphoreType.DMA((XCH,)),
        pltpu.SemaphoreType.DMA((4,)),
        pltpu.SemaphoreType.DMA((2, 2)),
        pltpu.SemaphoreType.DMA((2,)),
        pltpu.SemaphoreType.DMA((5,)),
        pltpu.SemaphoreType.DMA((S // RB,)),
        pltpu.SemaphoreType.DMA((2,)),
    ]
    out = pl.pallas_call(
        _kernel,
        out_shape=jax.ShapeDtypeStruct((S, D), BF),
        in_specs=[any_spec] * 11,
        out_specs=any_spec,
        scratch_shapes=scratch,
        compiler_params=pltpu.CompilerParams(vmem_limit_bytes=120 * 1024 * 1024),
    )(x, k, v, A_wq, A_wo, wr, B_w_gate, B_w_up, B_w_down, c, w_mod)
    return out.reshape(1, S, D)
```

```python
import functools
import math

import jax
import jax.numpy as jnp
from jax import lax
import jax.experimental.pallas as pl
import jax.experimental.pallas.tpu as pltpu

S = 2048
D = 1024
H = 32
DH = 128
F = 3584
EPS = 1e-5
QSCALE = (DH ** -0.5) * math.log2(math.e)

BQ = 256
RB = 256
RO = (512, 512, 512, 512)
NCH = 16
RC = 16
NSL = 4
XCH = 4
NEG = -3.0e38

BF = jnp.bfloat16
F32 = jnp.float32
NT = (((1,), (1,)), ((), ()))


def _ln(x):
    m = jnp.mean(x, axis=-1, keepdims=True)
    d = x - m
    v = jnp.mean(d * d, axis=-1, keepdims=True)
    return d * lax.rsqrt(v + EPS)


def _tiles(a, op):
    acc = a[:, 0:128]
    for t in range(1, a.shape[1] // 128):
        acc = op(acc, a[:, t * 128:(t + 1) * 128])
    return acc


def _recip(l):
    r = pl.reciprocal(l, approx=True)
    return r * (2.0 - l * r)


def _pack(a):
    return pltpu.bitcast(a, jnp.int32)


def _unpack(a):
    return pltpu.bitcast(a, BF)


def _half(start, size):
    return pl.ds(start // 2, size // 2)


def _kernel(x_hbm, k_hbm, v_hbm, wq_hbm, wo_hbm, wr_hbm, wg_hbm, wu_hbm, wd_hbm,
            c_hbm, wm_hbm, out_hbm,
            x_buf, h_buf, st_buf, wq_buf, k_buf, v_buf, o_buf, junk_buf, scol_buf, wo_buf, wg_buf,
            wu_buf, wd_buf, wm_buf, wmp_buf, mod_buf, mod2_buf, c_buf, wr_buf,
            fix_buf, sem_misc, sem_x, sem_wm, sem_kv, sem_wq, sem_wmp, sem_bg, sem_out,
            sem_fix):
    k_w, v_w, wq_w, wo_w, wmp_w = (r.bitcast(jnp.int32) for r in (k_buf, v_buf, wq_buf, wo_buf, wmp_buf))
    def cp_c():
        return pltpu.make_async_copy(c_hbm, c_buf, sem_misc.at[0])

    def cp_wr():
        return pltpu.make_async_copy(wr_hbm, wr_buf, sem_misc.at[1])

    def cp_wm(j):
        cols = pl.ds(j * 512, 512)
        return pltpu.make_async_copy(wm_hbm.at[:, cols], wm_buf.at[:, cols], sem_wm.at[j])

    XR = S // XCH

    def cp_x(j):
        rows = pl.ds(j * XR, XR)
        return pltpu.make_async_copy(x_hbm.at[rows, :], x_buf.at[rows, :], sem_x.at[j])

    def cp_k(h, slot):
        return pltpu.make_async_copy(k_hbm.at[h], k_buf.at[slot], sem_kv.at[0, slot])

    def cp_v(h, slot):
        return pltpu.make_async_copy(v_hbm.at[h], v_buf.at[slot], sem_kv.at[1, slot])

    def cp_wq(h, slot):
        cols = pl.ds(pl.multiple_of(h * DH, DH), DH)
        return pltpu.make_async_copy(wq_hbm.at[:, cols], wq_buf.at[slot], sem_wq.at[slot])

    def cp_wmp(h, slot=None):
        slot = h % NSL if slot is None else slot
        cols = pl.ds(pl.multiple_of(2 * D + h * DH, DH), DH)
        return pltpu.make_async_copy(wm_hbm.at[:, cols], wmp_buf.at[slot], sem_wmp.at[slot])

    def bg_copies(h):
        r32 = pl.ds(pl.multiple_of(h * 32, 32), 32)
        r112 = pl.ds(pl.multiple_of(h * 112, 16), 112)
        r128 = pl.ds(pl.multiple_of(h * 128, 128), 128)
        return [
            pltpu.make_async_copy(wo_hbm.at[r128, pl.ds(n * 128, 128)], wo_buf.at[n, r128, :], sem_bg.at[0])
            for n in range(D // 128)
        ] + [
            pltpu.make_async_copy(wg_hbm.at[r32, :], wg_buf.at[r32, :], sem_bg.at[2]),
            pltpu.make_async_copy(wu_hbm.at[r32, :], wu_buf.at[r32, :], sem_bg.at[3]),
            pltpu.make_async_copy(wd_hbm.at[r112, :], wd_buf.at[r112, :], sem_bg.at[4]),
        ]

    def bg_wait_all():
        pltpu.make_async_copy(wo_buf, wo_buf, sem_bg.at[0]).wait()
        pltpu.make_async_copy(wg_hbm, wg_buf, sem_bg.at[2]).wait()
        pltpu.make_async_copy(wu_hbm, wu_buf, sem_bg.at[3]).wait()
        pltpu.make_async_copy(wd_hbm, wd_buf, sem_bg.at[4]).wait()

    cp_c().start()
    cp_wm(0).start()
    cp_c().wait()
    for j in range(1, 4):
        cp_wm(j).start()
    cf = c_buf[...].astype(F32)
    sc = (cf * jax.nn.sigmoid(cf)).astype(BF)
    sc16 = jnp.broadcast_to(sc, (16, D))
    later = [
        [cp_wq(0, 0), cp_x(0)],
        [cp_x(1)],
        [cp_x(2)],
        [cp_x(3)],
    ]
    for j in range(4):
        cp_wm(j).wait()
        for cpy in later[j]:
            cpy.start()
        mj = jnp.dot(sc16, wm_buf[:, j * 512:(j + 1) * 512], preferred_element_type=F32)
        mod_buf[:, j * 512:(j + 1) * 512] = mj[0:8, :]

    scf = sc.astype(F32)
    for t in range(D // 128):
        scol_buf[t * 128:(t + 1) * 128, :] = jnp.broadcast_to(scf[:, t * 128:(t + 1) * 128], (128, 128)).T

    cp_wq(0, 0).wait()
    later = [
        [cp_k(0, 0)],
        [cp_v(0, 0)],
        [cp_wq(1, 1), cp_wmp(0), cp_wmp(1), cp_wmp(2)],
        [cp_wr()] + bg_copies(H - 1),
    ]
    for j in range(XCH):
        cp_x(j).wait()
        for cpy in later[j]:
            cpy.start()
        for t in range(XR // RB):
            rows = pl.ds(j * XR + t * RB, RB)
            n = _ln(x_buf[rows, :].astype(F32))
            h = n * (1.0 + mod_buf[0:1, D:2 * D]) + mod_buf[0:1, 0:D]
            hb = h.astype(BF)
            h_buf[_half(j * XR + t * RB, RB), :] = _pack(hb)
            q = jnp.dot(hb, _unpack(wq_w[0]), preferred_element_type=F32)
            o_buf[0, _half(j * XR + t * RB, RB), :] = _pack((q * QSCALE).astype(BF))

    def tie(a, t, zero):
        z = pltpu.bitcast(t, jnp.int32) & zero
        return jnp.concatenate([_unpack(_pack(a[0:16, :]) | z), a[16:, :]], axis=0)

    def qproj(h, slot, t, zero):
        hh = _unpack(h_buf[...])
        hh = jnp.concatenate([tie(hh[:, 0:128], t, zero), hh[:, 128:]], axis=1)
        q = jnp.dot(hh, _unpack(wq_w[slot]), preferred_element_type=F32)
        o_buf[h, :, :] = _pack((q * QSCALE).astype(BF))

    def mod_unit(h, i, acc):
        prod = _unpack(wmp_w[h % NSL, _half(i * 128, 128), :]).astype(F32) * scol_buf[i * 128:(i + 1) * 128, :]
        parts = [prod[t * 8:(t + 1) * 8, :] for t in range(16)]
        while len(parts) > 1:
            parts = [parts[t] + parts[t + 1] for t in range(0, len(parts), 2)]
        return parts[0] if acc is None else acc + parts[0]

    def tall(t):
        for _ in range(NCH):
            t = t + jnp.max(t, axis=1, keepdims=True)
        junk_buf[...] = t

    def attention(h, slot, zero):
        q_next = _unpack(o_buf[h, _half(0, BQ), :])
        for i in range(S // BQ):
            q = q_next
            if i > 0:
                q = tie(q, acc, zero)
            acc = mod_unit(h, i, acc if i else None)
            if i + 1 < S // BQ:
                q_next = _unpack(o_buf[h, _half((i + 1) * BQ, BQ), :])
            s = lax.dot_general(q, _unpack(k_w[slot]), NT, preferred_element_type=F32)
            m = jnp.max(_tiles(s, jnp.maximum), axis=1, keepdims=True)
            p = jnp.exp2(s - m)
            o = jnp.dot(p.astype(BF), _unpack(v_w[slot]), preferred_element_type=F32)
            l = jnp.sum(_tiles(p, jnp.add), axis=1, keepdims=True)
            o_buf[h, _half(i * BQ, BQ), :] = _pack((o * _recip(l)).astype(BF))
            if i == S // BQ - 1:
                tall(o[BQ - 8:, :])
        mod2_buf[h] = jnp.broadcast_to(jnp.sum(acc, axis=0, keepdims=True), (8, DH))
        return acc

    def head_body(h, carry):
        slot = lax.rem(h, 2)
        nslot = 1 - slot
        cp_k(h, slot).wait()
        cp_v(h, slot).wait()
        cp_wq(h + 1, nslot).wait()
        cp_wmp(h).wait()
        cp_k(h + 1, nslot).start()
        cp_v(h + 1, nslot).start()
        cp_wq(jnp.minimum(h + 2, H - 1), slot).start()
        acc = attention(h, slot, carry // H)
        qproj(h + 1, nslot, acc, carry // H)
        cp_wmp(jnp.minimum(h + 3, H - 1), (h + 3) % NSL).start()
        for cpy in bg_copies(h):
            cpy.start()
        return lax.rem(h, H)

    oz = lax.fori_loop(0, H - 1, head_body, 0) // H

    cp_wq(H - 1, (H - 2) % 2).wait()
    cp_k(H - 1, (H - 1) % 2).wait()
    cp_v(H - 1, (H - 1) % 2).wait()
    for hh in range(H - 1, H + 2):
        cp_wmp(H - 1, hh % NSL).wait()
    bg_wait_all()
    cp_wr().wait()
    attention(H - 1, (H - 1) % 2, oz)

    wr = wr_buf[...].astype(F32)

    def mod(i):
        base = (i - 2) * 8
        return jnp.concatenate([mod2_buf[base + t, 0:1, :] for t in range(8)], axis=1)

    ga, sb, cb1, gb = mod(2), mod(3), 1.0 + mod(4), mod(5)

    def cp_out(i):
        rows = pl.ds(sum(RO[:i]), RO[i])
        return pltpu.make_async_copy(st_buf.at[0, rows, :], out_hbm.at[rows, :], sem_out.at[i])

    def h2_of(x1):
        return (_ln(x1) * cb1 + sb).astype(BF).astype(F32)

    gai = pltpu.bitcast(ga, jnp.int32)

    sub = lax.broadcasted_iota(jnp.int32, (8, 128), 0)

    def epi_chunk(r0, yc, top, chain):
        rows = pl.ds(r0, RC)
        m1, i1, m2, i2 = top
        gac = ga
        if chain:
            zc = (i1 | i2) & oz
            gac = pltpu.bitcast(gai | jnp.concatenate([zc[0:1, :]] * (D // 128), axis=1), F32)
        x1 = x_buf[rows, :].astype(F32) + gac * yc
        h2 = h2_of(x1)
        st_buf[oz, rows, :] = (x1 + gb * h2).astype(BF)
        st_buf[oz + 1, rows, :] = h2.astype(BF)
        h2 = st_buf[oz + 1, rows, :].astype(F32)
        acc = h2[:, 0:128] * wr[0:1, :]
        for j in range(1, 8):
            acc = acc + h2[:, j * 128:(j + 1) * 128] * wr[j:j + 1, :]
        r = jnp.sum(acc, axis=1, keepdims=True).astype(BF).astype(F32)
        r = jnp.broadcast_to(r, (RC, 128))
        for u in range(RC // 8):
            ru, iu = r[u * 8:(u + 1) * 8, :], sub + (r0 + u * 8)
            gt1, gt2 = ru > m1, ru > m2
            m2 = jnp.where(gt1, m1, jnp.where(gt2, ru, m2))
            i2 = jnp.where(gt1, i1, jnp.where(gt2, iu, i2))
            m1 = jnp.where(gt1, ru, m1)
            i1 = jnp.where(gt1, iu, i1)
        return m1, i1, m2, i2

    starts = [sum(RO[:i]) for i in range(len(RO) + 1)]
    lowest = jnp.full((8, 128), -jnp.inf, F32)
    top = (lowest, sub, lowest, sub + 8)
    wo = jnp.concatenate([_unpack(wo_w[n]) for n in range(D // 128)], axis=1)
    y = None
    for i in range(len(RO) + 1):
        y_next = None
        if i < len(RO):
            oc = jnp.concatenate([_unpack(o_buf[hh, _half(starts[i], RO[i]), :]) for hh in range(H)], axis=1)
            y_next = jnp.dot(oc, wo, preferred_element_type=F32)
        if i > 0:
            for t in range(RO[i - 1] // RC):
                top = epi_chunk(starts[i - 1] + t * RC, y[t * RC:(t + 1) * RC, :], top, i < len(RO))
            cp_out(i - 1).start()
        y = y_next

    m1, i1, m2, i2 = top
    b1 = jnp.max(m1, axis=0, keepdims=True)
    j1 = jnp.min(jnp.where(m1 == b1, i1, S), axis=0, keepdims=True)
    taken = i1 == j1
    mr, ir = jnp.where(taken, m2, m1), jnp.where(taken, i2, i1)
    b2 = jnp.max(mr, axis=0, keepdims=True)
    j2 = jnp.min(jnp.where(mr == b2, ir, S), axis=0, keepdims=True)
    m1, m2 = b1, b2
    idx1 = jnp.clip(jnp.max(j1), 0, S - 1)
    idx2 = jnp.clip(jnp.max(j2), 0, S - 1)

    g1 = pl.multiple_of((idx1 // 16) * 16, 16)
    g2 = pl.multiple_of((idx2 // 16) * 16, 16)
    ri = lax.broadcasted_iota(jnp.int32, (16, D), 0)
    sel11 = ri == (idx1 - g1)
    sel22 = ri == (idx2 - g2)
    xs1 = jnp.sum(jnp.where(sel11, st_buf[1, pl.ds(g1, 16), :].astype(F32), 0.0), axis=0, keepdims=True)
    xs2 = jnp.sum(jnp.where(sel22, st_buf[1, pl.ds(g2, 16), :].astype(F32), 0.0), axis=0, keepdims=True)
    xsel = jnp.where(ri == 0, xs1, jnp.where(ri == 1, xs2, 0.0)).astype(BF)

    g = jnp.dot(xsel, wg_buf[...], preferred_element_type=F32)
    u = jnp.dot(xsel, wu_buf[...], preferred_element_type=F32)
    a = (g * jax.nn.sigmoid(g) * u).astype(BF)
    y = jnp.dot(a, wd_buf[...], preferred_element_type=F32)
    w1 = jax.nn.sigmoid(m1[:, 0:1])
    w2 = jax.nn.sigmoid(m2[:, 0:1])
    y1 = y[0:1, :] * w1
    y2 = y[1:2, :] * w2

    def fixed(gbase):
        upd = jnp.where(ri == (idx1 - gbase), y1, 0.0) + jnp.where(ri == (idx2 - gbase), y2, 0.0)
        return (st_buf[0, pl.ds(gbase, 16), :].astype(F32) + gb * upd).astype(BF)

    fix_buf[0] = fixed(g1)
    fix_buf[1] = fixed(g2)

    for i in range(len(RO)):
        cp_out(i).wait()

    cp1 = pltpu.make_async_copy(fix_buf.at[0], out_hbm.at[pl.ds(g1, 16), :], sem_fix.at[0])
    cp1.start()

    @pl.when(g1 != g2)
    def _():
        cp2 = pltpu.make_async_copy(fix_buf.at[1], out_hbm.at[pl.ds(g2, 16), :], sem_fix.at[1])
        cp2.start()
        cp2.wait()

    cp1.wait()


@jax.jit
def pallas_adaLN_cond__mha_block_cached__moe_arch_mod__prompt_kernel(
    A_x, A_k_cache, A_v_cache, A_wq, A_wo, B_x, B_w_r, B_w_gate, B_w_up, B_w_down, c, w_mod,
):
    del B_x
    x = A_x.reshape(S, D)
    k = A_k_cache.reshape(H, S, DH)
    v = A_v_cache.reshape(H, S, DH)
    wr = B_w_r.reshape(8, 128)
    any_spec = pl.BlockSpec(memory_space=pl.ANY)
    scratch = [
        pltpu.VMEM((S, D), BF),
        pltpu.VMEM((S // 2, D), jnp.int32),
        pltpu.VMEM((2, S, D), BF),
        pltpu.VMEM((2, D, DH), BF),
        pltpu.VMEM((2, S, DH), BF),
        pltpu.VMEM((2, S, DH), BF),
        pltpu.VMEM((H, S // 2, DH), jnp.int32),
        pltpu.VMEM((8, DH), F32),
        pltpu.VMEM((D, DH), F32),
        pltpu.VMEM((D // 128, H * DH, 128), BF),
        pltpu.VMEM((D, F), BF),
        pltpu.VMEM((D, F), BF),
        pltpu.VMEM((F, D), BF),
        pltpu.VMEM((D, 2 * D), BF),
        pltpu.VMEM((NSL, D, DH), BF),
        pltpu.VMEM((8, 2 * D), F32),
        pltpu.VMEM((H, 8, DH), F32),
        pltpu.VMEM((1, D), BF),
        pltpu.VMEM((8, 128), BF),
        pltpu.VMEM((2, 16, D), BF),
        pltpu.SemaphoreType.DMA((2,)),
        pltpu.SemaphoreType.DMA((XCH,)),
        pltpu.SemaphoreType.DMA((4,)),
        pltpu.SemaphoreType.DMA((2, 2)),
        pltpu.SemaphoreType.DMA((2,)),
        pltpu.SemaphoreType.DMA((NSL,)),
        pltpu.SemaphoreType.DMA((5,)),
        pltpu.SemaphoreType.DMA((len(RO),)),
        pltpu.SemaphoreType.DMA((2,)),
    ]
    out = pl.pallas_call(
        _kernel,
        out_shape=jax.ShapeDtypeStruct((S, D), BF),
        in_specs=[any_spec] * 11,
        out_specs=any_spec,
        scratch_shapes=scratch,
        compiler_params=pltpu.CompilerParams(vmem_limit_bytes=120 * 1024 * 1024),
    )(x, k, v, A_wq, A_wo, wr, B_w_gate, B_w_up, B_w_down, c, w_mod)
    return out.reshape(1, S, D)
```

```python
import functools
import math

import jax
import jax.numpy as jnp
from jax import lax
import jax.experimental.pallas as pl
import jax.experimental.pallas.tpu as pltpu

S = 2048
D = 1024
H = 32
DH = 128
F = 3584
EPS = 1e-5
QSCALE = (DH ** -0.5) * math.log2(math.e)

BQ = (304, 304, 288, 288, 288, 288, 288)
RB = 256
RO = (512, 512, 512, 512)
NCH = 16
RC = 16
NSL = 4
XCH = 4
NEG = -3.0e38

BF = jnp.bfloat16
F32 = jnp.float32
NT = (((1,), (1,)), ((), ()))


def _ln(x):
    m = jnp.mean(x, axis=-1, keepdims=True)
    d = x - m
    v = jnp.mean(d * d, axis=-1, keepdims=True)
    return d * lax.rsqrt(v + EPS)


def _tiles(a, op):
    acc = a[:, 0:128]
    for t in range(1, a.shape[1] // 128):
        acc = op(acc, a[:, t * 128:(t + 1) * 128])
    return acc


def _recip(l):
    r = pl.reciprocal(l, approx=True)
    return r * (2.0 - l * r)


def _pack(a):
    return pltpu.bitcast(a, jnp.int32)


def _unpack(a):
    return pltpu.bitcast(a, BF)


def _half(start, size):
    return pl.ds(start // 2, size // 2)


def _kernel(x_hbm, k_hbm, v_hbm, wq_hbm, wo_hbm, wr_hbm, wg_hbm, wu_hbm, wd_hbm,
            c_hbm, wm_hbm, out_hbm,
            x_buf, h_buf, st_buf, wq_buf, k_buf, v_buf, o_buf, junk_buf, scol_buf, wo_buf, wg_buf,
            wu_buf, wd_buf, wm_buf, wmp_buf, mod_buf, mod2_buf, c_buf, wr_buf,
            fix_buf, sem_misc, sem_x, sem_wm, sem_kv, sem_wq, sem_wmp, sem_bg, sem_out,
            sem_fix):
    k_w, v_w, wq_w, wo_w, wmp_w, h_w, o_w = (r.bitcast(jnp.int32) for r in (k_buf, v_buf, wq_buf, wo_buf, wmp_buf, h_buf, o_buf))
    def cp_c():
        return pltpu.make_async_copy(c_hbm, c_buf, sem_misc.at[0])

    def cp_wr():
        return pltpu.make_async_copy(wr_hbm, wr_buf, sem_misc.at[1])

    def cp_wm(j):
        cols = pl.ds(j * 512, 512)
        return pltpu.make_async_copy(wm_hbm.at[:, cols], wm_buf.at[:, cols], sem_wm.at[j])

    XR = S // XCH

    def cp_x(j):
        rows = pl.ds(j * XR, XR)
        return pltpu.make_async_copy(x_hbm.at[rows, :], x_buf.at[rows, :], sem_x.at[j])

    def cp_k(h, slot):
        return pltpu.make_async_copy(k_hbm.at[h], k_buf.at[slot], sem_kv.at[0, slot])

    def cp_v(h, slot):
        return pltpu.make_async_copy(v_hbm.at[h], v_buf.at[slot], sem_kv.at[1, slot])

    def cp_wq(h, slot):
        cols = pl.ds(pl.multiple_of(h * DH, DH), DH)
        return pltpu.make_async_copy(wq_hbm.at[:, cols], wq_buf.at[slot], sem_wq.at[slot])

    def cp_wmp(h, slot=None):
        slot = h % NSL if slot is None else slot
        cols = pl.ds(pl.multiple_of(2 * D + h * DH, DH), DH)
        return pltpu.make_async_copy(wm_hbm.at[:, cols], wmp_buf.at[slot], sem_wmp.at[slot])

    def bg_copies(h):
        r32 = pl.ds(pl.multiple_of(h * 32, 32), 32)
        r112 = pl.ds(pl.multiple_of(h * 112, 16), 112)
        r128 = pl.ds(pl.multiple_of(h * 128, 128), 128)
        return [
            pltpu.make_async_copy(wo_hbm.at[r128, pl.ds(n * 128, 128)], wo_buf.at[n, r128, :], sem_bg.at[0])
            for n in range(D // 128)
        ] + [
            pltpu.make_async_copy(wg_hbm.at[r32, :], wg_buf.at[r32, :], sem_bg.at[2]),
            pltpu.make_async_copy(wu_hbm.at[r32, :], wu_buf.at[r32, :], sem_bg.at[3]),
            pltpu.make_async_copy(wd_hbm.at[r112, :], wd_buf.at[r112, :], sem_bg.at[4]),
        ]

    def bg_wait_all():
        wo_all = wo_buf.at[:, pl.ds(0, H * DH), :]
        pltpu.make_async_copy(wo_all, wo_all, sem_bg.at[0]).wait()
        cp_wr().wait()

    def expert_wait():
        pltpu.make_async_copy(wg_hbm, wg_buf, sem_bg.at[2]).wait()
        pltpu.make_async_copy(wu_hbm, wu_buf, sem_bg.at[3]).wait()
        pltpu.make_async_copy(wd_hbm, wd_buf, sem_bg.at[4]).wait()

    cp_c().start()
    cp_wm(0).start()
    wo_buf[0, H * DH:, :] = jnp.zeros((16, 128), BF)
    cp_c().wait()
    for j in range(1, 4):
        cp_wm(j).start()
    cf = c_buf[...].astype(F32)
    sc = (cf * jax.nn.sigmoid(cf)).astype(BF)
    sc16 = jnp.broadcast_to(sc, (16, D))
    later = [
        [cp_wq(0, 0), cp_x(0)],
        [cp_x(1)],
        [cp_x(2)],
        [cp_x(3)],
    ]
    for j in range(4):
        cp_wm(j).wait()
        for cpy in later[j]:
            cpy.start()
        mj = jnp.dot(sc16, wm_buf[:, j * 512:(j + 1) * 512], preferred_element_type=F32)
        mod_buf[:, j * 512:(j + 1) * 512] = mj[0:8, :]

    scf = sc.astype(F32)
    for t in range(D // 128):
        scol_buf[t * 128:(t + 1) * 128, :] = jnp.broadcast_to(scf[:, t * 128:(t + 1) * 128], (128, 128)).T

    cp_wq(0, 0).wait()
    later = [
        [cp_k(0, 0)],
        [cp_v(0, 0)],
        [cp_wq(1, 1), cp_wmp(0), cp_wmp(1), cp_wmp(2)],
        [cp_wr()] + bg_copies(H - 1),
    ]
    for j in range(XCH):
        cp_x(j).wait()
        for cpy in later[j]:
            cpy.start()
        for t in range(XR // RB):
            rows = pl.ds(j * XR + t * RB, RB)
            n = _ln(x_buf[rows, :].astype(F32))
            h = n * (1.0 + mod_buf[0:1, D:2 * D]) + mod_buf[0:1, 0:D]
            hb = h.astype(BF)
            for n in range(D // 128):
                h_buf[n, rows, :] = hb[:, n * 128:(n + 1) * 128]
            q = jnp.dot(hb, _unpack(wq_w[0]), preferred_element_type=F32)
            o_buf[0, rows, :] = (q * QSCALE).astype(BF)

    def tie(a, t, zero):
        z = pltpu.bitcast(t, jnp.int32) & zero
        return jnp.concatenate([_unpack(_pack(a[0:16, :]) | z), a[16:, :]], axis=0)

    def qproj(h, slot, t, zero):
        hh = [_unpack(h_w[n]) for n in range(D // 128)]
        hh = jnp.concatenate([tie(hh[0], t, zero)] + hh[1:], axis=1)
        q = jnp.dot(hh, _unpack(wq_w[slot]), preferred_element_type=F32)
        o_buf[h, :, :] = (q * QSCALE).astype(BF)

    def mod_unit(h, i, acc):
        per = 8 // len(BQ)
        for j in range(i * per, 8 if i == len(BQ) - 1 else (i + 1) * per):
            acc = mod_unit1(h, j, acc)
        return acc

    def mod_unit1(h, i, acc):
        prod = _unpack(wmp_w[h % NSL, _half(i * 128, 128), :]).astype(F32) * scol_buf[i * 128:(i + 1) * 128, :]
        parts = [prod[t * 8:(t + 1) * 8, :] for t in range(16)]
        while len(parts) > 1:
            parts = [parts[t] + parts[t + 1] for t in range(0, len(parts), 2)]
        return parts[0] if acc is None else acc + parts[0]

    def tall(t):
        for _ in range(NCH):
            t = t + jnp.max(t, axis=1, keepdims=True)
        junk_buf[...] = t

    def attention(h, slot, zero):
        st = [sum(BQ[:i]) for i in range(len(BQ))]
        q_next = _unpack(o_w[h, _half(0, BQ[0]), :])
        for i in range(len(BQ)):
            q = q_next
            if i > 0:
                q = tie(q, acc, zero)
            acc = mod_unit(h, i, acc if i else None)
            if i + 1 < len(BQ):
                q_next = _unpack(o_w[h, _half(st[i + 1], BQ[i + 1]), :])
            s = lax.dot_general(q, _unpack(k_w[slot]), NT, preferred_element_type=F32)
            m = jnp.max(_tiles(s, jnp.maximum), axis=1, keepdims=True)
            p = jnp.exp2(s - m)
            o = jnp.dot(p.astype(BF), _unpack(v_w[slot]), preferred_element_type=F32)
            l = jnp.sum(_tiles(p, jnp.add), axis=1, keepdims=True)
            o_buf[h, pl.ds(st[i], BQ[i]), :] = (o * _recip(l)).astype(BF)
            if i == len(BQ) - 1:
                tall(o[BQ[i] - 8:, :])
        mj = jnp.broadcast_to(jnp.sum(acc, axis=0, keepdims=True), (8, DH))
        mod2_buf[h] = mj
        return mj

    def head_body(h, carry):
        slot = lax.rem(h, 2)
        nslot = 1 - slot
        cp_k(h, slot).wait()
        cp_v(h, slot).wait()
        cp_wq(h + 1, nslot).wait()
        cp_wmp(h).wait()
        cp_k(h + 1, nslot).start()
        cp_v(h + 1, nslot).start()
        cp_wq(jnp.minimum(h + 2, H - 1), slot).start()
        for cpy in bg_copies(h):
            cpy.start()
        cp_wmp(jnp.minimum(h + 3, H - 1), (h + 3) % NSL).start()
        zero = wo_w[0, H * DH // 2:, :]
        acc = attention(h, slot, zero)
        qproj(h + 1, nslot, acc, zero)
        return carry

    lax.fori_loop(0, H - 1, head_body, 0)
    oz = wo_w[0, H * DH // 2:, :]

    cp_wq(H - 1, (H - 2) % 2).wait()
    cp_k(H - 1, (H - 1) % 2).wait()
    cp_v(H - 1, (H - 1) % 2).wait()
    for hh in range(H - 1, H + 2):
        cp_wmp(H - 1, hh % NSL).wait()
    bg_wait_all()
    attention(H - 1, (H - 1) % 2, oz)

    wr = wr_buf[...].astype(F32)

    def mod(i):
        base = (i - 2) * 8
        return jnp.concatenate([mod2_buf[base + t, 0:1, :] for t in range(8)], axis=1)

    ga, sb, cb1, gb = mod(2), mod(3), 1.0 + mod(4), mod(5)

    def cp_out(i):
        rows = pl.ds(sum(RO[:i]), RO[i])
        return pltpu.make_async_copy(st_buf.at[0, rows, :], out_hbm.at[rows, :], sem_out.at[i])

    def h2_of(x1):
        return (_ln(x1) * cb1 + sb).astype(BF).astype(F32)

    gai = pltpu.bitcast(ga, jnp.int32)

    sub = lax.broadcasted_iota(jnp.int32, (8, 128), 0)

    def epi_chunk(r0, yc, top, chain):
        rows = pl.ds(r0, RC)
        m1, i1, m2, i2 = top
        gac = ga
        if chain:
            zc = (i1 | i2) & oz
            gac = pltpu.bitcast(gai | jnp.concatenate([zc[0:1, :]] * (D // 128), axis=1), F32)
        x1 = x_buf[rows, :].astype(F32) + gac * yc
        h2 = h2_of(x1)
        st_buf[0, rows, :] = (x1 + gb * h2).astype(BF)
        st_buf[1, rows, :] = h2.astype(BF)
        acc = h2[:, 0:128] * wr[0:1, :]
        for j in range(1, 8):
            acc = acc + h2[:, j * 128:(j + 1) * 128] * wr[j:j + 1, :]
        r = jnp.sum(acc, axis=1, keepdims=True).astype(BF).astype(F32)
        r = jnp.broadcast_to(r, (RC, 128))
        for u in range(RC // 8):
            ru, iu = r[u * 8:(u + 1) * 8, :], sub + (r0 + u * 8)
            gt1, gt2 = ru > m1, ru > m2
            m2 = jnp.where(gt1, m1, jnp.where(gt2, ru, m2))
            i2 = jnp.where(gt1, i1, jnp.where(gt2, iu, i2))
            m1 = jnp.where(gt1, ru, m1)
            i1 = jnp.where(gt1, iu, i1)
        return m1, i1, m2, i2

    starts = [sum(RO[:i]) for i in range(len(RO) + 1)]
    lowest = jnp.full((8, 128), -jnp.inf, F32)
    top = (lowest, sub, lowest, sub + 8)
    wo = jnp.concatenate([_unpack(wo_w[n, 0:H * DH // 2, :]) for n in range(D // 128)], axis=1)
    y = None
    for i in range(len(RO) + 1):
        y_next = None
        if i < len(RO):
            oc = jnp.concatenate([_unpack(o_w[hh, _half(starts[i], RO[i]), :]) for hh in range(H)], axis=1)
            y_next = jnp.dot(oc, wo, preferred_element_type=F32)
        if i > 0:
            for t in range(RO[i - 1] // RC):
                top = epi_chunk(starts[i - 1] + t * RC, y[t * RC:(t + 1) * RC, :], top, i < len(RO))
            cp_out(i - 1).start()
        y = y_next

    m1, i1, m2, i2 = top
    b1 = jnp.max(m1, axis=0, keepdims=True)
    j1 = jnp.min(jnp.where(m1 == b1, i1, S), axis=0, keepdims=True)
    taken = i1 == j1
    mr, ir = jnp.where(taken, m2, m1), jnp.where(taken, i2, i1)
    b2 = jnp.max(mr, axis=0, keepdims=True)
    j2 = jnp.min(jnp.where(mr == b2, ir, S), axis=0, keepdims=True)
    m1, m2 = b1, b2
    idx1 = jnp.clip(jnp.max(j1), 0, S - 1)
    idx2 = jnp.clip(jnp.max(j2), 0, S - 1)

    expert_wait()
    g1 = pl.multiple_of((idx1 // 16) * 16, 16)
    g2 = pl.multiple_of((idx2 // 16) * 16, 16)
    ri = lax.broadcasted_iota(jnp.int32, (16, D), 0)
    sel11 = ri == (idx1 - g1)
    sel22 = ri == (idx2 - g2)
    xs1 = jnp.sum(jnp.where(sel11, st_buf[1, pl.ds(g1, 16), :].astype(F32), 0.0), axis=0, keepdims=True)
    xs2 = jnp.sum(jnp.where(sel22, st_buf[1, pl.ds(g2, 16), :].astype(F32), 0.0), axis=0, keepdims=True)
    xsel = jnp.where(ri == 0, xs1, jnp.where(ri == 1, xs2, 0.0)).astype(BF)

    g = jnp.dot(xsel, wg_buf[...], preferred_element_type=F32)
    u = jnp.dot(xsel, wu_buf[...], preferred_element_type=F32)
    a = (g * jax.nn.sigmoid(g) * u).astype(BF)
    y = jnp.dot(a, wd_buf[...], preferred_element_type=F32)
    w1 = jax.nn.sigmoid(m1[:, 0:1])
    w2 = jax.nn.sigmoid(m2[:, 0:1])
    y1 = y[0:1, :] * w1
    y2 = y[1:2, :] * w2

    def fixed(gbase):
        upd = jnp.where(ri == (idx1 - gbase), y1, 0.0) + jnp.where(ri == (idx2 - gbase), y2, 0.0)
        return (st_buf[0, pl.ds(gbase, 16), :].astype(F32) + gb * upd).astype(BF)

    fix_buf[0] = fixed(g1)
    fix_buf[1] = fixed(g2)

    for i in range(len(RO)):
        cp_out(i).wait()

    cp1 = pltpu.make_async_copy(fix_buf.at[0], out_hbm.at[pl.ds(g1, 16), :], sem_fix.at[0])
    cp1.start()

    @pl.when(g1 != g2)
    def _():
        cp2 = pltpu.make_async_copy(fix_buf.at[1], out_hbm.at[pl.ds(g2, 16), :], sem_fix.at[1])
        cp2.start()
        cp2.wait()

    cp1.wait()


@jax.jit
def pallas_adaLN_cond__mha_block_cached__moe_arch_mod__prompt_kernel(
    A_x, A_k_cache, A_v_cache, A_wq, A_wo, B_x, B_w_r, B_w_gate, B_w_up, B_w_down, c, w_mod,
):
    del B_x
    x = A_x.reshape(S, D)
    k = A_k_cache.reshape(H, S, DH)
    v = A_v_cache.reshape(H, S, DH)
    wr = B_w_r.reshape(8, 128)
    any_spec = pl.BlockSpec(memory_space=pl.ANY)
    scratch = [
        pltpu.VMEM((S, D), BF),
        pltpu.VMEM((D // 128, S, 128), BF),
        pltpu.VMEM((2, S, D), BF),
        pltpu.VMEM((2, D, DH), BF),
        pltpu.VMEM((2, S, DH), BF),
        pltpu.VMEM((2, S, DH), BF),
        pltpu.VMEM((H, S, DH), BF),
        pltpu.VMEM((8, DH), F32),
        pltpu.VMEM((D, DH), F32),
        pltpu.VMEM((D // 128, H * DH + 16, 128), BF),
        pltpu.VMEM((D, F), BF),
        pltpu.VMEM((D, F), BF),
        pltpu.VMEM((F, D), BF),
        pltpu.VMEM((D, 2 * D), BF),
        pltpu.VMEM((NSL, D, DH), BF),
        pltpu.VMEM((8, 2 * D), F32),
        pltpu.VMEM((H, 8, DH), F32),
        pltpu.VMEM((1, D), BF),
        pltpu.VMEM((8, 128), BF),
        pltpu.VMEM((2, 16, D), BF),
        pltpu.SemaphoreType.DMA((2,)),
        pltpu.SemaphoreType.DMA((XCH,)),
        pltpu.SemaphoreType.DMA((4,)),
        pltpu.SemaphoreType.DMA((2, 2)),
        pltpu.SemaphoreType.DMA((2,)),
        pltpu.SemaphoreType.DMA((NSL,)),
        pltpu.SemaphoreType.DMA((5,)),
        pltpu.SemaphoreType.DMA((len(RO),)),
        pltpu.SemaphoreType.DMA((2,)),
    ]
    out = pl.pallas_call(
        _kernel,
        out_shape=jax.ShapeDtypeStruct((S, D), BF),
        in_specs=[any_spec] * 11,
        out_specs=any_spec,
        scratch_shapes=scratch,
        compiler_params=pltpu.CompilerParams(vmem_limit_bytes=120 * 1024 * 1024),
    )(x, k, v, A_wq, A_wo, wr, B_w_gate, B_w_up, B_w_down, c, w_mod)
    return out.reshape(1, S, D)
```

```python
import functools
import math

import jax
import jax.numpy as jnp
from jax import lax
import jax.experimental.pallas as pl
import jax.experimental.pallas.tpu as pltpu

S = 2048
D = 1024
H = 32
DH = 128
F = 3584
EPS = 1e-5
QSCALE = (DH ** -0.5) * math.log2(math.e)

BQ = (304, 304, 288, 288, 288, 288, 288)
RB = 64
RO = (896, 704, 320, 128)
NCH = 16
RC = 16
NSL = 4
EXTRA = 0
XR = (256,) * 8
NEG = -3.0e38

BF = jnp.bfloat16
F32 = jnp.float32
NT = (((1,), (1,)), ((), ()))


def _ln(x):
    m = jnp.mean(x, axis=-1, keepdims=True)
    d = x - m
    v = jnp.mean(d * d, axis=-1, keepdims=True)
    return d * lax.rsqrt(v + EPS)


def _tiles(a, op):
    acc = a[:, 0:128]
    for t in range(1, a.shape[1] // 128):
        acc = op(acc, a[:, t * 128:(t + 1) * 128])
    return acc


def _recip(l):
    r = pl.reciprocal(l, approx=True)
    return r * (2.0 - l * r)


def _pack(a):
    return pltpu.bitcast(a, jnp.int32)


def _unpack(a):
    return pltpu.bitcast(a, BF)


def _half(start, size):
    return pl.ds(start // 2, size // 2)


def _kernel(x_hbm, k_hbm, v_hbm, wq_hbm, wo_hbm, wr_hbm, wg_hbm, wu_hbm, wd_hbm,
            c_hbm, wm_hbm, out_hbm,
            x_buf, h_buf, st_buf, h2_buf, wq_buf, k_buf, v_buf, o_buf, junk_buf, scol_buf, wo_buf, wg_buf,
            wu_buf, wd_buf, wm_buf, wmp_buf, mod_buf, mod2_buf, c_buf, wr_buf,
            fix_buf, sem_misc, sem_x, sem_wm, sem_kv, sem_wq, sem_wmp, sem_bg, sem_out,
            sem_fix):
    k_w, v_w, wq_w, wo_w, wmp_w, h_w, o_w, x_w, wg_w, wu_w, wd_w = (r.bitcast(jnp.int32) for r in (k_buf, v_buf, wq_buf, wo_buf, wmp_buf, h_buf, o_buf, x_buf, wg_buf, wu_buf, wd_buf))
    def cp_c():
        return pltpu.make_async_copy(c_hbm, c_buf, sem_misc.at[0])

    def cp_wr():
        return pltpu.make_async_copy(wr_hbm, wr_buf, sem_misc.at[1])

    def cp_wm(j):
        cols = pl.ds(j * 512, 512)
        return pltpu.make_async_copy(wm_hbm.at[:, cols], wm_buf.at[:, cols], sem_wm.at[j])

    def cp_x(j):
        rows = pl.ds(sum(XR[:j]), XR[j])
        return [pltpu.make_async_copy(x_hbm.at[rows, pl.ds(n * 128, 128)], x_buf.at[n, rows, :], sem_x.at[j])
                for n in range(D // 128)]

    def wait_x(j):
        dst = x_buf.at[:, pl.ds(sum(XR[:j]), XR[j]), :]
        pltpu.make_async_copy(dst, dst, sem_x.at[j]).wait()

    def load_x(r0, n):
        return jnp.concatenate([_unpack(x_w[t, _half(r0, n), :]) for t in range(D // 128)], axis=1).astype(F32)

    def cp_k(h, slot):
        return pltpu.make_async_copy(k_hbm.at[h], k_buf.at[slot], sem_kv.at[0, slot])

    def cp_v(h, slot):
        return pltpu.make_async_copy(v_hbm.at[h], v_buf.at[slot], sem_kv.at[1, slot])

    def cp_wq(h, slot):
        cols = pl.ds(pl.multiple_of(h * DH, DH), DH)
        return pltpu.make_async_copy(wq_hbm.at[:, cols], wq_buf.at[slot], sem_wq.at[slot])

    def cp_wmp(h, slot=None):
        slot = h % NSL if slot is None else slot
        cols = pl.ds(pl.multiple_of(2 * D + h * DH, DH), DH)
        return pltpu.make_async_copy(wm_hbm.at[:, cols], wmp_buf.at[slot], sem_wmp.at[slot])

    def bg_copies(h):
        cg = pl.ds(pl.multiple_of(jnp.minimum(h, F // 128 - 1) * 128, 128), 128)
        rd = pl.ds(pl.multiple_of(h // 8 * (F // 4), 128), F // 4)
        cd = pl.ds(pl.multiple_of(h % 8 * 128, 128), 128)
        r128 = pl.ds(pl.multiple_of(h * 128, 128), 128)
        return [
            pltpu.make_async_copy(wo_hbm.at[r128, pl.ds(n * 128, 128)], wo_buf.at[n, r128, :], sem_bg.at[0])
            for n in range(D // 128)
        ] + [
            pltpu.make_async_copy(wg_hbm.at[:, cg], wg_buf.at[h], sem_bg.at[2]),
            pltpu.make_async_copy(wu_hbm.at[:, cg], wu_buf.at[h], sem_bg.at[3]),
            pltpu.make_async_copy(wd_hbm.at[rd, cd], wd_buf.at[h % 8, rd, :], sem_bg.at[4]),
        ]

    def bg_wait_all():
        wo_all = wo_buf.at[:, pl.ds(0, H * DH), :]
        pltpu.make_async_copy(wo_all, wo_all, sem_bg.at[0]).wait()
        cp_wr().wait()

    def expert_wait():
        pltpu.make_async_copy(wg_buf, wg_buf, sem_bg.at[2]).wait()
        pltpu.make_async_copy(wu_buf, wu_buf, sem_bg.at[3]).wait()
        pltpu.make_async_copy(wd_buf, wd_buf, sem_bg.at[4]).wait()

    cp_c().start()
    cp_wm(0).start()
    wo_buf[0, H * DH:, :] = jnp.zeros((16, 128), BF)
    cp_c().wait()
    for j in range(1, 4):
        cp_wm(j).start()
    cf = c_buf[...].astype(F32)
    sc = (cf * jax.nn.sigmoid(cf)).astype(BF)
    sc16 = jnp.broadcast_to(sc, (16, D))
    queue = ([[cp_wq(0, 0)]] + [cp_x(j) for j in range(len(XR))]
             + [[cp_k(0, 0)], [cp_v(0, 0)], [cp_wq(1, 1), cp_wmp(0)],
                [cp_wmp(1), cp_wmp(2), cp_wr()] + bg_copies(H - 1)])

    def issue(n):
        for _ in range(n):
            if queue:
                for cpy in queue.pop(0):
                    cpy.start()

    for j in range(4):
        cp_wm(j).wait()
        issue((1, 1, 1, 2)[j])
        mj = jnp.dot(sc16, wm_buf[:, j * 512:(j + 1) * 512], preferred_element_type=F32)
        mod_buf[:, j * 512:(j + 1) * 512] = mj[0:8, :]

    scf = sc.astype(F32)
    for t in range(D // 128):
        scol_buf[t * 128:(t + 1) * 128, :] = jnp.broadcast_to(scf[:, t * 128:(t + 1) * 128], (128, 128)).T

    cp_wq(0, 0).wait()
    def qproj0(j):
        rows = pl.ds(sum(XR[:j]), XR[j])
        hh = jnp.concatenate([_unpack(h_w[n, _half(sum(XR[:j]), XR[j]), :]) for n in range(D // 128)], axis=1)
        q = jnp.dot(hh, _unpack(wq_w[0]), preferred_element_type=F32)
        o_buf[0, rows, :] = (q * QSCALE).astype(BF)

    for j in range(len(XR)):
        wait_x(j)
        issue(2 if j >= len(XR) - EXTRA else 1)
        if j > 0:
            qproj0(j - 1)
        for t in range(XR[j] // RB):
            r0 = sum(XR[:j]) + t * RB
            rows = pl.ds(r0, RB)
            h = _ln(load_x(r0, RB)) * (1.0 + mod_buf[0:1, D:2 * D]) + mod_buf[0:1, 0:D]
            hb = h.astype(BF)
            for n in range(D // 128):
                h_buf[n, rows, :] = hb[:, n * 128:(n + 1) * 128]
    qproj0(len(XR) - 1)
    assert not queue

    def tie(a, t, zero):
        z = pltpu.bitcast(t, jnp.int32) & zero
        return jnp.concatenate([_unpack(_pack(a[0:16, :]) | z), a[16:, :]], axis=0)

    def qproj(h, slot, t, zero):
        hh = [_unpack(h_w[n]) for n in range(D // 128)]
        hh = jnp.concatenate([tie(hh[0], t, zero)] + hh[1:], axis=1)
        q = jnp.dot(hh, _unpack(wq_w[slot]), preferred_element_type=F32)
        o_buf[h, :, :] = (q * QSCALE).astype(BF)

    def mod_unit(h, i, acc):
        per = 8 // len(BQ)
        for j in range(i * per, 8 if i == len(BQ) - 1 else (i + 1) * per):
            acc = mod_unit1(h, j, acc)
        return acc

    def mod_unit1(h, i, acc):
        prod = _unpack(wmp_w[h % NSL, _half(i * 128, 128), :]).astype(F32) * scol_buf[i * 128:(i + 1) * 128, :]
        parts = [prod[t * 8:(t + 1) * 8, :] for t in range(16)]
        while len(parts) > 1:
            parts = [parts[t] + parts[t + 1] for t in range(0, len(parts), 2)]
        return parts[0] if acc is None else acc + parts[0]

    def tall(t):
        for _ in range(NCH):
            t = t + jnp.max(t, axis=1, keepdims=True)
        junk_buf[...] = t

    def attention(h, slot, zero):
        st = [sum(BQ[:i]) for i in range(len(BQ))]
        q_next = _unpack(o_w[h, _half(0, BQ[0]), :])
        for i in range(len(BQ)):
            q = q_next
            if i > 0:
                q = tie(q, acc, zero)
            acc = mod_unit(h, i, acc if i else None)
            if i + 1 < len(BQ):
                q_next = _unpack(o_w[h, _half(st[i + 1], BQ[i + 1]), :])
            s = lax.dot_general(q, _unpack(k_w[slot]), NT, preferred_element_type=F32)
            m = jnp.max(_tiles(s, jnp.maximum), axis=1, keepdims=True)
            p = jnp.exp2(s - m)
            o = jnp.dot(p.astype(BF), _unpack(v_w[slot]), preferred_element_type=F32)
            l = jnp.sum(_tiles(p, jnp.add), axis=1, keepdims=True)
            o_buf[h, pl.ds(st[i], BQ[i]), :] = (o * _recip(l)).astype(BF)
            if i == len(BQ) - 1:
                tall(o[BQ[i] - 8:, :])
        mj = jnp.broadcast_to(jnp.sum(acc, axis=0, keepdims=True), (8, DH))
        mod2_buf[h] = mj
        return mj

    def head_body(h, carry):
        slot = lax.rem(h, 2)
        nslot = 1 - slot
        cp_k(h, slot).wait()
        cp_v(h, slot).wait()
        cp_wq(h + 1, nslot).wait()
        cp_wmp(h).wait()
        cp_k(h + 1, nslot).start()
        cp_v(h + 1, nslot).start()
        cp_wq(jnp.minimum(h + 2, H - 1), slot).start()
        for cpy in bg_copies(h):
            cpy.start()
        cp_wmp(jnp.minimum(h + 3, H - 1), (h + 3) % NSL).start()
        zero = wo_w[0, H * DH // 2:, :]
        acc = attention(h, slot, zero)
        qproj(h + 1, nslot, acc, zero)
        return carry

    lax.fori_loop(0, H - 1, head_body, 0)
    oz = wo_w[0, H * DH // 2:, :]

    cp_wq(H - 1, (H - 2) % 2).wait()
    cp_k(H - 1, (H - 1) % 2).wait()
    cp_v(H - 1, (H - 1) % 2).wait()
    for hh in range(H - 1, H + 2):
        cp_wmp(H - 1, hh % NSL).wait()
    bg_wait_all()
    attention(H - 1, (H - 1) % 2, oz)

    wr = wr_buf[...].astype(F32)

    def mod(i):
        base = (i - 2) * 8
        return jnp.concatenate([mod2_buf[base + t, 0:1, :] for t in range(8)], axis=1)

    ga, sb, cb1, gb = mod(2), mod(3), 1.0 + mod(4), mod(5)

    def cp_out(i):
        rows = pl.ds(sum(RO[:i]), RO[i])
        return [pltpu.make_async_copy(st_buf.at[n, rows, :], out_hbm.at[rows, pl.ds(n * 128, 128)], sem_out.at[i])
                for n in range(D // 128)]

    def h2_of(x1):
        return (_ln(x1) * cb1 + sb).astype(BF).astype(F32)

    gai = pltpu.bitcast(ga, jnp.int32)

    sub = lax.broadcasted_iota(jnp.int32, (8, 128), 0)

    def epi_chunk(r0, yc, top, chain):
        rows = pl.ds(r0, RC)
        m1, i1, m2, i2 = top
        gac = ga
        if chain:
            zc = (i1 | i2) & oz
            gac = pltpu.bitcast(gai | jnp.concatenate([zc[0:1, :]] * (D // 128), axis=1), F32)
        x1 = load_x(r0, RC) + gac * yc
        h2 = h2_of(x1)
        ob = (x1 + gb * h2).astype(BF)
        for n in range(D // 128):
            st_buf[n, rows, :] = ob[:, n * 128:(n + 1) * 128]
            h2_buf[rows, n * 128:(n + 1) * 128] = h2[:, n * 128:(n + 1) * 128]
        acc = h2[:, 0:128] * wr[0:1, :]
        for j in range(1, 8):
            acc = acc + h2[:, j * 128:(j + 1) * 128] * wr[j:j + 1, :]
        r = jnp.sum(acc, axis=1, keepdims=True).astype(BF).astype(F32)
        r = jnp.broadcast_to(r, (RC, 128))
        for u in range(RC // 8):
            ru, iu = r[u * 8:(u + 1) * 8, :], sub + (r0 + u * 8)
            gt1, gt2 = ru > m1, ru > m2
            m2 = jnp.where(gt1, m1, jnp.where(gt2, ru, m2))
            i2 = jnp.where(gt1, i1, jnp.where(gt2, iu, i2))
            m1 = jnp.where(gt1, ru, m1)
            i1 = jnp.where(gt1, iu, i1)
        return m1, i1, m2, i2

    starts = [sum(RO[:i]) for i in range(len(RO) + 1)]
    lowest = jnp.full((8, 128), -jnp.inf, F32)
    top = (lowest, sub, lowest, sub + 8)
    wo = jnp.concatenate([_unpack(wo_w[n, 0:H * DH // 2, :]) for n in range(D // 128)], axis=1)
    y = None
    for i in range(len(RO) + 1):
        y_next = None
        if i < len(RO):
            oc = jnp.concatenate([_unpack(o_w[hh, _half(starts[i], RO[i]), :]) for hh in range(H)], axis=1)
            y_next = jnp.dot(oc, wo, preferred_element_type=F32)
        if i > 0:
            for t in range(RO[i - 1] // RC):
                top = epi_chunk(starts[i - 1] + t * RC, y[t * RC:(t + 1) * RC, :], top, i < len(RO))
            for cpy in cp_out(i - 1):
                cpy.start()
        y = y_next

    m1, i1, m2, i2 = top
    b1 = jnp.max(m1, axis=0, keepdims=True)
    j1 = jnp.min(jnp.where(m1 == b1, i1, S), axis=0, keepdims=True)
    taken = i1 == j1
    mr, ir = jnp.where(taken, m2, m1), jnp.where(taken, i2, i1)
    b2 = jnp.max(mr, axis=0, keepdims=True)
    j2 = jnp.min(jnp.where(mr == b2, ir, S), axis=0, keepdims=True)
    m1, m2 = b1, b2
    idx1 = jnp.clip(jnp.max(j1), 0, S - 1)
    idx2 = jnp.clip(jnp.max(j2), 0, S - 1)

    expert_wait()
    g1 = pl.multiple_of((idx1 // 16) * 16, 16)
    g2 = pl.multiple_of((idx2 // 16) * 16, 16)
    ri = lax.broadcasted_iota(jnp.int32, (16, D), 0)
    sel11 = ri == (idx1 - g1)
    sel22 = ri == (idx2 - g2)
    xs1 = jnp.sum(jnp.where(sel11, h2_buf[pl.ds(g1, 16), :], 0.0), axis=0, keepdims=True)
    xs2 = jnp.sum(jnp.where(sel22, h2_buf[pl.ds(g2, 16), :], 0.0), axis=0, keepdims=True)
    xsel = jnp.where(ri == 0, xs1, jnp.where(ri == 1, xs2, 0.0)).astype(BF)

    wg, wu, wd = (jnp.concatenate([_unpack(w[n]) for n in range(nt)], axis=1)
                  for w, nt in ((wg_w, F // 128), (wu_w, F // 128), (wd_w, D // 128)))
    g = jnp.dot(xsel, wg, preferred_element_type=F32)
    u = jnp.dot(xsel, wu, preferred_element_type=F32)
    a = (g * jax.nn.sigmoid(g) * u).astype(BF)
    y = (jnp.dot(a[:, :F // 2], wd[:F // 2, :], preferred_element_type=F32)
         + jnp.dot(a[:, F // 2:], wd[F // 2:, :], preferred_element_type=F32))
    w1 = jax.nn.sigmoid(m1[:, 0:1])
    w2 = jax.nn.sigmoid(m2[:, 0:1])
    y1 = y[0:1, :] * w1
    y2 = y[1:2, :] * w2

    def fixed(gbase):
        upd = jnp.where(ri == (idx1 - gbase), y1, 0.0) + jnp.where(ri == (idx2 - gbase), y2, 0.0)
        base = jnp.concatenate([st_buf[n, pl.ds(gbase, 16), :] for n in range(D // 128)], axis=1)
        return (base.astype(F32) + gb * upd).astype(BF)

    fix_buf[0] = fixed(g1)
    fix_buf[1] = fixed(g2)

    for i in range(len(RO)):
        for cpy in cp_out(i):
            cpy.wait()

    cp1 = pltpu.make_async_copy(fix_buf.at[0], out_hbm.at[pl.ds(g1, 16), :], sem_fix.at[0])
    cp1.start()

    @pl.when(g1 != g2)
    def _():
        cp2 = pltpu.make_async_copy(fix_buf.at[1], out_hbm.at[pl.ds(g2, 16), :], sem_fix.at[1])
        cp2.start()
        cp2.wait()

    cp1.wait()


@jax.jit
def pallas_adaLN_cond__mha_block_cached__moe_arch_mod__prompt_kernel(
    A_x, A_k_cache, A_v_cache, A_wq, A_wo, B_x, B_w_r, B_w_gate, B_w_up, B_w_down, c, w_mod,
):
    del B_x
    x = A_x.reshape(S, D)
    k = A_k_cache.reshape(H, S, DH)
    v = A_v_cache.reshape(H, S, DH)
    wr = B_w_r.reshape(8, 128)
    any_spec = pl.BlockSpec(memory_space=pl.ANY)
    scratch = [
        pltpu.VMEM((D // 128, S, 128), BF),
        pltpu.VMEM((D // 128, S, 128), BF),
        pltpu.VMEM((D // 128, S, 128), BF),
        pltpu.VMEM((S, D), F32),
        pltpu.VMEM((2, D, DH), BF),
        pltpu.VMEM((2, S, DH), BF),
        pltpu.VMEM((2, S, DH), BF),
        pltpu.VMEM((H, S, DH), BF),
        pltpu.VMEM((8, DH), F32),
        pltpu.VMEM((D, DH), F32),
        pltpu.VMEM((D // 128, H * DH + 16, 128), BF),
        pltpu.VMEM((H, D, 128), BF),
        pltpu.VMEM((H, D, 128), BF),
        pltpu.VMEM((D // 128, F, 128), BF),
        pltpu.VMEM((D, 2 * D), BF),
        pltpu.VMEM((NSL, D, DH), BF),
        pltpu.VMEM((8, 2 * D), F32),
        pltpu.VMEM((H, 8, DH), F32),
        pltpu.VMEM((1, D), BF),
        pltpu.VMEM((8, 128), BF),
        pltpu.VMEM((2, 16, D), BF),
        pltpu.SemaphoreType.DMA((2,)),
        pltpu.SemaphoreType.DMA((len(XR),)),
        pltpu.SemaphoreType.DMA((4,)),
        pltpu.SemaphoreType.DMA((2, 2)),
        pltpu.SemaphoreType.DMA((2,)),
        pltpu.SemaphoreType.DMA((NSL,)),
        pltpu.SemaphoreType.DMA((5,)),
        pltpu.SemaphoreType.DMA((len(RO),)),
        pltpu.SemaphoreType.DMA((2,)),
    ]
    out = pl.pallas_call(
        _kernel,
        out_shape=jax.ShapeDtypeStruct((S, D), BF),
        in_specs=[any_spec] * 11,
        out_specs=any_spec,
        scratch_shapes=scratch,
        compiler_params=pltpu.CompilerParams(vmem_limit_bytes=120 * 1024 * 1024),
    )(x, k, v, A_wq, A_wo, wr, B_w_gate, B_w_up, B_w_down, c, w_mod)
    return out.reshape(1, S, D)
```
